```python
import os as _os
_os.environ.setdefault("JAX_PLATFORMS", "cpu")
import jax
import jax.numpy as jnp

def _softmax(x, axis=-1):
    return jax.nn.softmax(x, axis=axis)
def _gelu(x):
    return jax.nn.gelu(x, approximate=True)
def _silu(x):
    return jax.nn.silu(x)
def _sigmoid(x):
    return jax.nn.sigmoid(x)
def _layernorm(x, axis=-1, eps=1e-5):
    m = jnp.mean(x, axis=axis, keepdims=True)
    v = jnp.var(x, axis=axis, keepdims=True)
    return (x - m) / jnp.sqrt(v + eps)
def _scatter_add(tgt, idx, src, axis=0):
    return tgt.at[idx].add(src)
def _segment_sum(src, seg, n):
    return jax.ops.segment_sum(src, seg, n)
class _Rng:
    def __init__(self, key):
        self._k = key
    def _next(self):
        self._k, sub = jax.random.split(self._k)
        return sub
    def normal(self, shape):
        return jax.random.normal(self._next(), shape, dtype=jnp.bfloat16)
    def randint(self, lo, hi, shape):
        return jax.random.randint(self._next(), shape, lo, hi, dtype=jnp.int32)
    def uniform(self, shape, lo=0.0, hi=1.0):
        return jax.random.uniform(self._next(), shape, jnp.bfloat16, lo, hi)
    def permutation(self, n):
        return jax.random.permutation(self._next(), n)


kernel_name = 'standalone__gqa_block_cached__near_ridge'

def setup_inputs():
    _rng = _Rng(jax.random.key(int.from_bytes(__import__("os").urandom(4), "little")))
    _w = (lambda a: (lambda t: t.astype(jnp.bfloat16) if jnp.issubdtype(t.dtype, jnp.floating) else t)(jnp.asarray(a)))
    B, Sq, D = 8, 96, 448
    Hq, Hkv, Sk, Dh = 16, 8, 2048, 256
    assert Hq % Hkv == 0, (Hq, Hkv)
    return {
        "x": _w((lambda *s: _rng.normal(s) * 0.8)(B, Sq, D)),
        "k_cache": _w((lambda *s: _rng.normal(s) * 0.8)(B, Hkv, Sk, Dh)),
        "v_cache": _w((lambda *s: _rng.normal(s) * 0.05)(B, Hkv, Sk, Dh)),
        "wq": _w((lambda *s: _rng.normal(s) * 0.8)(D, Hq * Dh) * (D ** -0.5)),
        "wo": _w((lambda *s: _rng.normal(s) * 0.05)(Hq * Dh, D) * ((Hq * Dh) ** -0.5)),
    }

def reference(x, k_cache, v_cache, wq, wo):
    B, Sq, D = x.shape
    Hq, Dh = 16, 256
    Hkv = k_cache.shape[1]
    rep = Hq // Hkv
    q = (lambda x, *d: x.transpose(*d))((x @ wq).reshape(B, Sq, Hq, Dh), 0, 2, 1, 3)
    k = jnp.repeat(k_cache, rep, axis=1)
    v = jnp.repeat(v_cache, rep, axis=1)
    scores = jnp.einsum("bhqd,bhkd->bhqk", q, k) * (Dh ** -0.5)
    p = _softmax(scores, axis=-1)
    o = jnp.einsum("bhqk,bhkd->bhqd", p, v)
    return (lambda x, *d: x.transpose(*d))(o, 0, 2, 1, 3).reshape(B, Sq, Hq * Dh) @ wo
```

```python
import functools, math
import jax, jax.numpy as jnp, numpy as np
from jax import lax
import jax.experimental.pallas as pl
import jax.experimental.pallas.tpu as pltpu

def make(W=4, CH=256, B=8, Sq=96, D=448, Hkv=8, Sk=2048, Dh=256, rep=2, vmem=64, flags=None,
         prio=0, nodma=False, lag=2, qpos=0, nobc=True, opos=0, midissue=4, lastsplit=1, nocompute=False):
    M = 2*Sq
    NP = B // 2
    NSUP = NP*Hkv
    NU = NSUP*2
    NIT = NU*2
    R = 8
    assert 2 <= W <= R-2
    c = (Dh ** -0.5) * math.log2(math.e)
    HW = rep*Dh
    NC = Sk // CH
    NT = (((1,),(1,)),((),()))
    shr = lambda a, n: a >> n
    def kern(x_hbm, k_hbm, v_hbm, wq_hbm, wo_hbm, o_hbm, x_v, wq_v, wo_v, ring, q_s, acc, ost, oc_s, sem_kv, sem_l, sem_w, sem_o):
        def item_copy(j_s, j_t):
            s = shr(j_s, 1); r = j_s & 1
            h = shr(s, 2); bp = s & 3
            src = (k_hbm if j_t == 0 else v_hbm).at[2*bp + r, h]
            slot = (2*j_s + j_t) & (R-1)
            return pltpu.make_async_copy(src, ring.at[slot], sem_kv.at[slot])
        def issue(u, t, static):
            du, t2 = divmod(t + W, 2)
            if static and 2*u + t + W >= NIT_main: return
            if nodma: return
            item_copy(u + du, t2).start(priority=(t2 % 2) if prio else 0)
        def item_wait(u, t):
            if not nodma: item_copy(u, t).wait()
        LP = Sk // lastsplit
        def last_copy(t, i):
            src = (k_hbm if t == 0 else v_hbm).at[B-1, Hkv-1, pl.ds(i*LP, LP)]
            slot = (2*(NU-1) + t) & (R-1)
            return pltpu.make_async_copy(src, ring.at[slot, pl.ds(i*LP, LP)], sem_l.at[t*lastsplit + i])
        NIT_main = NIT - 2 if lastsplit > 1 else NIT
        def wq_copy(h):
            return pltpu.make_async_copy(wq_hbm.at[:, pl.ds(pl.multiple_of(h*HW, HW), HW)], wq_v.at[h], sem_w.at[1+h])
        def wo_copy(h):
            return pltpu.make_async_copy(wo_hbm.at[:, pl.ds(pl.multiple_of(h*HW, HW), HW)], wo_v.at[h], sem_w.at[1+Hkv+h])
        cx = pltpu.make_async_copy(x_hbm, x_v, sem_w.at[0])
        cx.start(); wq_copy(0).start()
        item_copy(0, 0).start(); item_copy(0, 1).start()
        cx.wait(); wq_copy(0).wait()
        for j in range(2, W):
            item_copy(j // 2, j % 2).start()
        wo_copy(0).start(); wq_copy(1).start()
        if nodma:
            for j in range(W): item_copy(j // 2, j % 2).wait()

        def qproj(s):
            h = shr(s, 2); bp = s & 3
            xr = x_v[pl.ds(pl.multiple_of(bp*M, M), M), :]
            q = jnp.dot(xr, wq_v[h], preferred_element_type=jnp.float32)
            q = (q * c).astype(jnp.bfloat16)
            q_s[0, 0:Sq, :] = q[0:Sq, 0:Dh]
            q_s[0, Sq:M, :] = q[0:Sq, Dh:HW]
            q_s[1, 0:Sq, :] = q[Sq:M, 0:Dh]
            q_s[1, Sq:M, :] = q[Sq:M, Dh:HW]

        def lanefold(a, acc_, op):
            for i in range(a.shape[1] // 128):
                sl = a[:, i*128:(i+1)*128]
                acc_ = sl if acc_ is None else op(acc_, sl)
            return acc_

        def out_copy(bp):
            return pltpu.make_async_copy(ost.at[bp], o_hbm.at[pl.ds(pl.multiple_of(bp*M, M), M)], sem_o.at[bp])

        def outproj(s, static):
            h = shr(s, 2); bp = s & 3
            r = lax.dot_general(oc_s[...], wo_v[h], NT, preferred_element_type=jnp.float32)
            tot = jnp.where(h == 0, r, acc[bp] + r)
            acc[bp] = tot
            if static:
                if h == Hkv - 1:
                    ost[bp] = tot.astype(ost.dtype)
                    out_copy(bp).start()
            else:
                ost[bp] = tot.astype(ost.dtype)
                pl.when(h == Hkv - 1)(lambda: out_copy(bp).start())

        def unit(s, r, static):
            u = 2*s + r
            h = shr(s, 2); bp = s & 3
            last = static and (u == NU - 1) and lastsplit > 1
            Kr = ring.at[(2*u) & (R-1)]; Vr = ring.at[(2*u + 1) & (R-1)]
            if not last:
                item_wait(u, 0); item_wait(u, 1)
            if r == 0:
                def f():
                    wo_copy(h).wait()
                    if static:
                        if h + 1 < Hkv: wo_copy(h + 1).start()
                    else:
                        pl.when(h + 1 < Hkv)(lambda: wo_copy(h + 1).start())
                if static:
                    if s >= 1 and bp == 1: f()
                else:
                    pl.when(bp == 1)(f)
            else:
                def g():
                    wq_copy(h + 1).wait()
                    if static:
                        if h + 2 < Hkv: wq_copy(h + 2).start()
                    else:
                        pl.when(h + 2 < Hkv)(lambda: wq_copy(h + 2).start())
                if static:
                    if bp == 3 and h + 1 < Hkv: g()
                else:
                    pl.when(jnp.logical_and(bp == 3, h + 1 < Hkv))(g)
            issue(u, 0, static)
            if nocompute:
                issue(u, 1, static)
                if last:
                    for i in range(lastsplit):
                        last_copy(0, i).wait(); last_copy(1, i).wait()
                return
            S = {}
            st = dict(m=None, ls=None, o=None)
            def do_qk(cc):
                if last and (cc * CH) % LP == 0: last_copy(0, cc * CH // LP).wait()
                S[cc] = lax.dot_general(q_s[r], Kr[cc*CH:(cc+1)*CH, :], NT, preferred_element_type=jnp.float32)
            def do_smpv(cc):
                v = S.pop(cc); t = st
                cm = jnp.max(lanefold(v, None, jnp.maximum), axis=1, keepdims=True)
                mnew = cm if t['m'] is None else jnp.maximum(t['m'], cm)
                p = jnp.exp2(v - mnew)
                ps = lanefold(p, None, jnp.add)
                if last and (cc * CH) % LP == 0: last_copy(1, cc * CH // LP).wait()
                pvv = jnp.dot(p.astype(jnp.bfloat16), Vr[cc*CH:(cc+1)*CH, :], preferred_element_type=jnp.float32)
                if t['m'] is None:
                    t['ls'] = ps; t['o'] = pvv
                else:
                    alpha = jnp.exp2(t['m'] - mnew)
                    t['ls'] = t['ls'] * alpha + ps
                    t['o'] = t['o'] * alpha + pvv
                t['m'] = mnew
            do_next = (not static) or s + 1 < NSUP
            do_prev = (not static) or s > 0
            if r == 0 and opos == 0 and do_prev: outproj(s - 1, static)
            for i in range(NC + lag):
                if i < NC: do_qk(i)
                if r == 0 and opos == 1 and i == 0 and do_prev: outproj(s - 1, static)
                if i == midissue: issue(u, 1, static)
                j = i - lag
                if r == 1 and j == NC - 1 and qpos == 0 and do_next: qproj(s + 1)
                if j >= 0: do_smpv(j)
            if r == 1 and qpos == 1 and do_next: qproj(s + 1)
            l = jnp.sum(st['ls'], axis=1, keepdims=True)
            on = (st['o'] * (1.0 / l)).astype(jnp.bfloat16)
            oc_s[r*Sq:(r+1)*Sq, 0:Dh] = on[0:Sq]
            oc_s[r*Sq:(r+1)*Sq, Dh:HW] = on[Sq:M]

        def body(s, static):
            unit(s, 0, static)
            unit(s, 1, static)

        qproj(0)
        nmain = (NIT_main - W - 4) // 4 + 1
        while 2*(2*(nmain-1)+1) + 1 + W >= NIT_main: nmain -= 1
        body(0, True)
        def lb(s, carry):
            body(s, False)
            return carry
        lax.fori_loop(1, nmain, lb, 0)
        for s in range(nmain, NSUP):
            if lastsplit > 1 and s == NSUP - 1:
                pass
            body(s, True)
        if nocompute:
            return
        outproj(NSUP - 1, True)
        for bp in range(NP): out_copy(bp).wait()

    def f(x, k, v, wq, wo):
        x2 = x.reshape(B*Sq, D)
        woT = wo.T
        HBM = pl.BlockSpec(memory_space=pltpu.HBM)
        out = pl.pallas_call(
            kern,
            in_specs=[HBM]*5,
            out_specs=HBM,
            out_shape=jax.ShapeDtypeStruct((B*Sq, D), jnp.bfloat16),
            scratch_shapes=[
                pltpu.VMEM((B*Sq, D), jnp.bfloat16),
                pltpu.VMEM((Hkv, D, HW), jnp.bfloat16),
                pltpu.VMEM((Hkv, D, HW), jnp.bfloat16),
                pltpu.VMEM((R, Sk, Dh), jnp.bfloat16),
                pltpu.VMEM((2, M, Dh), jnp.bfloat16),
                pltpu.VMEM((NP, M, D), jnp.float32),
                pltpu.VMEM((NP, M, D), jnp.bfloat16),
                pltpu.VMEM((M, HW), jnp.bfloat16),
                pltpu.SemaphoreType.DMA((R,)),
                pltpu.SemaphoreType.DMA((2*lastsplit,)),
                pltpu.SemaphoreType.DMA((1 + 2*Hkv,)),
                pltpu.SemaphoreType.DMA((NP,)),
            ],
            compiler_params=pltpu.CompilerParams(vmem_limit_bytes=vmem*1024*1024, flags=flags, disable_bounds_checks=nobc),
        )(x2, k, v, wq, woT)
        return out.reshape(B, Sq, D)
    return f


@jax.jit
def pallas_standalone__gqa_block_cached__near_ridge_kernel(x, k_cache, v_cache, wq, wo):
    return make(W=4, CH=256, lag=1)(x, k_cache, v_cache, wq, wo)
```

```python
import math
import jax
import jax.numpy as jnp
from jax import lax
import jax.experimental.pallas as pl
import jax.experimental.pallas.tpu as pltpu

_REP = 2
_CH = 256
_RING = 8
_WINDOW = 4
_NT = (((1,), (1,)), ((), ()))


def _lanefold(a, op):
    out = a[:, 0:128]
    for i in range(1, a.shape[1] // 128):
        out = op(out, a[:, i * 128:(i + 1) * 128])
    return out


def _make_kernel(B, Sq, D, Hkv, Sk, Dh):
    M = 2 * Sq
    NP = B // 2
    NSUP = NP * Hkv
    NU = 2 * NSUP
    NIT = 2 * NU
    HW = _REP * Dh
    NC = Sk // _CH
    W = _WINDOW
    R = _RING
    assert NP == 4 and Sk % _CH == 0
    qscale = (Dh ** -0.5) * math.log2(math.e)

    def kernel(x_hbm, k_hbm, v_hbm, wq_hbm, wo_hbm, o_hbm,
               x_v, wq_v, wo_v, ring, q_s, acc, ost, oc_s,
               sem_kv, sem_w, sem_o):

        def kv_copy(u, t):
            s = u >> 1
            src = (k_hbm if t == 0 else v_hbm).at[2 * (s & 3) + (u & 1), s >> 2]
            slot = (2 * u + t) & (R - 1)
            return pltpu.make_async_copy(src, ring.at[slot], sem_kv.at[slot])

        def issue(u, t, static):
            if static and 2 * u + t + W >= NIT:
                return
            du, t2 = divmod(t + W, 2)
            kv_copy(u + du, t2).start(priority=1)

        def wq_copy(h):
            return pltpu.make_async_copy(
                wq_hbm.at[:, pl.ds(pl.multiple_of(h * HW, HW), HW)], wq_v.at[h], sem_w.at[1 + h])

        def wo_copy(h):
            return pltpu.make_async_copy(
                wo_hbm.at[:, pl.ds(pl.multiple_of(h * HW, HW), HW)], wo_v.at[h],
                sem_w.at[1 + Hkv + h])

        def out_copy(bp):
            return pltpu.make_async_copy(ost.at[bp], o_hbm.at[pl.ds(bp * M, M)], sem_o.at[bp])

        def half_copy(r):
            bp = NP - 1
            return pltpu.make_async_copy(
                ost.at[bp, pl.ds(r * Sq, Sq)], o_hbm.at[pl.ds(bp * M + r * Sq, Sq)],
                sem_o.at[NP - 1 + r])

        x_copy = pltpu.make_async_copy(x_hbm, x_v, sem_w.at[0])
        x_copy.start()
        wq_copy(0).start()
        kv_copy(0, 0).start(priority=1)
        kv_copy(0, 1).start(priority=1)
        x_copy.wait()
        wq_copy(0).wait()
        for j in range(2, W):
            kv_copy(j // 2, j % 2).start(priority=1)
        wo_copy(0).start()
        wq_copy(1).start()

        def qproj(s):
            xr = x_v[pl.ds(pl.multiple_of((s & 3) * M, M), M), :]
            q = jnp.dot(xr, wq_v[s >> 2], preferred_element_type=jnp.float32)
            q = (q * qscale).astype(jnp.bfloat16)
            q_s[0, 0:Sq, :] = q[0:Sq, 0:Dh]
            q_s[0, Sq:M, :] = q[0:Sq, Dh:HW]
            q_s[1, 0:Sq, :] = q[Sq:M, 0:Dh]
            q_s[1, Sq:M, :] = q[Sq:M, Dh:HW]

        def outproj(s):
            h = s >> 2
            bp = s & 3
            r = lax.dot_general(oc_s[...], wo_v[h], _NT, preferred_element_type=jnp.float32)
            tot = jnp.where(h == 0, r, acc[bp] + r)
            acc[bp] = tot
            ost[bp] = tot.astype(ost.dtype)

        def half_outproj(r):
            bp = NP - 1
            rows = slice(r * Sq, (r + 1) * Sq)
            rr = lax.dot_general(oc_s[rows, :], wo_v[Hkv - 1], _NT,
                                 preferred_element_type=jnp.float32)
            ost[bp, rows, :] = (acc[bp, rows, :] + rr).astype(ost.dtype)
            half_copy(r).start()

        def when(static, cond, fn):
            if static:
                if cond:
                    fn()
            else:
                pl.when(cond)(fn)

        def unit(s, r, static):
            u = 2 * s + r
            h = s >> 2
            bp = s & 3
            k_ref = ring.at[(2 * u) & (R - 1)]
            v_ref = ring.at[(2 * u + 1) & (R - 1)]
            kv_copy(u, 0).wait()
            kv_copy(u, 1).wait()

            if r == 0:
                def wo_step():
                    wo_copy(h).wait()
                    when(static, h + 1 < Hkv, lambda: wo_copy(h + 1).start())
                when(static, bp == 1, wo_step)
            else:
                def wq_step():
                    wq_copy(h + 1).wait()
                    when(static, h + 2 < Hkv, lambda: wq_copy(h + 2).start())
                if static:
                    when(True, bp == 3 and h + 1 < Hkv, wq_step)
                else:
                    when(False, jnp.logical_and(bp == 3, h + 1 < Hkv), wq_step)
            issue(u, 0, static)
            last = static and u == NU - 1
            if last:
                for b in range(NP - 1):
                    out_copy(b).start()

            scores = {}
            st = dict(m=None, l=None, o=None)

            def do_qk(cc):
                scores[cc] = lax.dot_general(
                    q_s[r], k_ref[cc * _CH:(cc + 1) * _CH, :], _NT,
                    preferred_element_type=jnp.float32)

            def do_softmax_pv(cc):
                sc = scores.pop(cc)
                cm = jnp.max(_lanefold(sc, jnp.maximum), axis=1, keepdims=True)
                m_new = cm if st['m'] is None else jnp.maximum(st['m'], cm)
                p = jnp.exp2(sc - m_new)
                ps = _lanefold(p, jnp.add)
                pv = jnp.dot(p.astype(jnp.bfloat16), v_ref[cc * _CH:(cc + 1) * _CH, :],
                             preferred_element_type=jnp.float32)
                if st['m'] is None:
                    st['l'] = ps
                    st['o'] = pv
                else:
                    alpha = jnp.exp2(st['m'] - m_new)
                    st['l'] = st['l'] * alpha + ps
                    st['o'] = st['o'] * alpha + pv
                st['m'] = m_new

            if r == 0 and ((not static) or s > 0):
                outproj(s - 1)
            for i in range(NC + 1):
                if i < NC:
                    do_qk(i)
                if i == 1:
                    issue(u, 1, static)
                    if last:
                        half_outproj(0)
                if i >= 1:
                    do_softmax_pv(i - 1)
            if r == 1 and ((not static) or s + 1 < NSUP):
                qproj(s + 1)
            l = jnp.sum(st['l'], axis=1, keepdims=True)
            on = (st['o'] * (1.0 / l)).astype(jnp.bfloat16)
            oc_s[r * Sq:(r + 1) * Sq, 0:Dh] = on[0:Sq]
            oc_s[r * Sq:(r + 1) * Sq, Dh:HW] = on[Sq:M]

        def body(s, static):
            unit(s, 0, static)
            unit(s, 1, static)

        qproj(0)
        nmain = NSUP
        while 2 * (2 * (nmain - 1) + 1) + 1 + W >= NIT:
            nmain -= 1
        body(0, True)

        def loop_body(s, carry):
            body(s, False)
            return carry
        lax.fori_loop(1, nmain, loop_body, 0)
        for s in range(nmain, NSUP):
            body(s, True)
        half_outproj(1)
        for b in range(NP - 1):
            out_copy(b).wait()
        half_copy(0).wait()
        half_copy(1).wait()

    return kernel


@jax.jit
def pallas_standalone__gqa_block_cached__near_ridge_kernel(
    x: jax.Array,
    k_cache: jax.Array,
    v_cache: jax.Array,
    wq: jax.Array,
    wo: jax.Array,
):
    B, Sq, D = x.shape
    _, Hkv, Sk, Dh = k_cache.shape
    M = 2 * Sq
    NP = B // 2
    HW = _REP * Dh
    hbm = pl.BlockSpec(memory_space=pltpu.HBM)
    out = pl.pallas_call(
        _make_kernel(B, Sq, D, Hkv, Sk, Dh),
        in_specs=[hbm] * 5,
        out_specs=hbm,
        out_shape=jax.ShapeDtypeStruct((B * Sq, D), x.dtype),
        scratch_shapes=[
            pltpu.VMEM((B * Sq, D), jnp.bfloat16),
            pltpu.VMEM((Hkv, D, HW), jnp.bfloat16),
            pltpu.VMEM((Hkv, D, HW), jnp.bfloat16),
            pltpu.VMEM((_RING, Sk, Dh), jnp.bfloat16),
            pltpu.VMEM((2, M, Dh), jnp.bfloat16),
            pltpu.VMEM((NP, M, D), jnp.float32),
            pltpu.VMEM((NP, M, D), x.dtype),
            pltpu.VMEM((M, HW), jnp.bfloat16),
            pltpu.SemaphoreType.DMA((_RING,)),
            pltpu.SemaphoreType.DMA((1 + 2 * Hkv,)),
            pltpu.SemaphoreType.DMA((NP + 1,)),
        ],
        compiler_params=pltpu.CompilerParams(
            vmem_limit_bytes=64 * 1024 * 1024, disable_bounds_checks=True),
    )(x.reshape(B * Sq, D), k_cache, v_cache, wq, wo.T)
    return out.reshape(B, Sq, D)
```
